```python
import jax
import jax.numpy as jnp

def _softmax(x, axis=-1):
    return jax.nn.softmax(x, axis=axis)
def _gelu(x):
    return jax.nn.gelu(x, approximate=True)
def _silu(x):
    return jax.nn.silu(x)
def _sigmoid(x):
    return jax.nn.sigmoid(x)
def _layernorm(x, axis=-1, eps=1e-5):
    m = jnp.mean(x, axis=axis, keepdims=True)
    v = jnp.var(x, axis=axis, keepdims=True)
    return (x - m) / jnp.sqrt(v + eps)
def _scatter_add(tgt, idx, src, axis=0):
    return tgt.at[idx].add(src)
def _segment_sum(src, seg, n):
    return jax.ops.segment_sum(src, seg, n)
class _Rng:
    def __init__(self, key):
        self._k = key
    def _next(self):
        self._k, sub = jax.random.split(self._k)
        return sub
    def normal(self, shape):
        return jax.random.normal(self._next(), shape, dtype=jnp.bfloat16)
    def randint(self, lo, hi, shape):
        return jax.random.randint(self._next(), shape, lo, hi, dtype=jnp.int32)
    def uniform(self, shape, lo=0.0, hi=1.0):
        return jax.random.uniform(self._next(), shape, jnp.bfloat16, lo, hi)
    def permutation(self, n):
        return jax.random.permutation(self._next(), n)


kernel_name = 'gated_mix__sliding_block_cached__dense_activation_gelu__decode'

def setup_inputs():
    _rng = _Rng(jax.random.key(int.from_bytes(__import__("os").urandom(4), "little")))
    _w = (lambda a: (lambda t: t.astype(jnp.bfloat16) if jnp.issubdtype(t.dtype, jnp.floating) else t)(jnp.asarray(a)))
    def _A_setup():
        B, Sq, D = 1, 1, 640
        Hq, Hkv, Sk, Dh = 32, 32, 32768, 192
        assert Hq % Hkv == 0, (Hq, Hkv)
        return {
            "x": _w((lambda *s: _rng.normal(s) * 0.05)(B, Sq, D)),
            "k_cache": _w((lambda *s: _rng.normal(s) * 0.05)(B, Hkv, Sk, Dh)),
            "v_cache": _w((lambda *s: _rng.normal(s) * 0.05)(B, Hkv, Sk, Dh)),
            "wq": _w((lambda *s: _rng.normal(s) * 0.05)(D, Hq * Dh) * (D ** -0.5)),
            "wo": _w((lambda *s: _rng.normal(s) * 0.05)(Hq * Dh, D) * ((Hq * Dh) ** -0.5)),
        }
    _A_in = _A_setup()

    def _B_setup():
        B, S, D, F = 1, 1, 640, 1536
        return {
            "x": _w((lambda *s: _rng.normal(s) * 0.05)(B, S, D)),
            "w1": _w((lambda *s: _rng.normal(s) * 0.05)(D, F) * (D ** -0.5)),
            "b1": _w((lambda *s: _rng.normal(s) * 0.05)(F) * 0.01),
            "w2": _w((lambda *s: _rng.normal(s) * 0.05)(F, D) * (F ** -0.5)),
            "b2": _w((lambda *s: _rng.normal(s) * 0.05)(D) * 0.01),
        }
    _B_in = _B_setup()

    return {
        "A_x": _A_in["x"],
        "A_k_cache": _A_in["k_cache"],
        "A_v_cache": _A_in["v_cache"],
        "A_wq": _A_in["wq"],
        "A_wo": _A_in["wo"],
        "B_x": _B_in["x"],
        "B_w1": _B_in["w1"],
        "B_b1": _B_in["b1"],
        "B_w2": _B_in["w2"],
        "B_b2": _B_in["b2"],
        "gate_w": _w((lambda *s: _rng.normal(s) * 0.05)(640)),
    }

def reference(A_x, A_k_cache, A_v_cache, A_wq, A_wo, B_x, B_w1, B_b1, B_w2, B_b2, gate_w):
    def _A_ref(x, k_cache, v_cache, wq, wo):
        B, Sq, D = x.shape
        Hq, Dh = 32, 192
        Hkv, Sk = k_cache.shape[1], k_cache.shape[2]
        W = min(4096, max(256, Sk // 4))
        rep = Hq // Hkv
        q = (lambda x, *d: x.transpose(*d))((x @ wq).reshape(B, Sq, Hq, Dh), 0, 2, 1, 3)
        k = jnp.repeat(k_cache[:, :, Sk - W:, :], rep, axis=1)
        v = jnp.repeat(v_cache[:, :, Sk - W:, :], rep, axis=1)
        scores = jnp.einsum("bhqd,bhkd->bhqk", q, k) * (Dh ** -0.5)
        p = _softmax(scores, axis=-1)
        o = jnp.einsum("bhqk,bhkd->bhqd", p, v)
        return (lambda x, *d: x.transpose(*d))(o, 0, 2, 1, 3).reshape(B, Sq, Hq * Dh) @ wo

    def _B_ref(x, w1, b1, w2, b2):
        h = jnp.einsum("bsd,df->bsf", x, w1) + b1
        h = _gelu(h)
        return jnp.einsum("bsf,fd->bsd", h, w2) + b2

    x = A_x
    g = _sigmoid((x * gate_w).sum(-1, keepdims=True))
    a = _A_ref(x, A_k_cache, A_v_cache, A_wq, A_wo)
    b = _B_ref(x, B_w1, B_b1, B_w2, B_b2)
    return g * a + (1 - g) * b
```

```python
import jax
import jax.numpy as jnp
import jax.experimental.pallas as pl
import jax.experimental.pallas.tpu as pltpu

_BF16 = jnp.bfloat16
_F32 = jnp.float32


def _gelu(x):
    c = 0.7978845608028654
    return 0.5 * x * (1.0 + jnp.tanh(c * (x + 0.044715 * (x * x * x))))


@jax.jit
def pallas_gated_mix__sliding_block_cached__dense_activation_gelu__decode_kernel(
    A_x: jax.Array,
    A_k_cache: jax.Array,
    A_v_cache: jax.Array,
    A_wq: jax.Array,
    A_wo: jax.Array,
    B_x: jax.Array,
    B_w1: jax.Array,
    B_b1: jax.Array,
    B_w2: jax.Array,
    B_b2: jax.Array,
    gate_w: jax.Array,
):
    D = A_x.shape[-1]
    _, H, SK, DH = A_k_cache.shape
    F = B_w1.shape[1]
    W = min(4096, max(256, SK // 4))
    NBUF = 3
    CD, CS = 16, 2048
    chunks = [(d0, s0) for d0 in range(0, DH, CD) for s0 in range(0, W, CS)]
    scale = DH ** -0.5

    def kernel(x_hbm, gw_hbm, b1_hbm, b2_hbm, k_hbm, v_hbm, wq_hbm, wo_hbm, w1_hbm, w2_hbm,
               o_ref,
               x_v, gw_v, b1_v, b2_v, wq_v, wo_v, w1_v, w2_v, kbuf, vbuf, q_scr, sem_s, sem_kv):
        c_x, c_gw, c_b1, c_b2, c_wq, c_wo, c_w1, c_w2 = [
            pltpu.make_async_copy(s, d, sem_s.at[i]) for i, (s, d) in enumerate(
                [(x_hbm, x_v), (gw_hbm, gw_v), (b1_hbm, b1_v), (b2_hbm, b2_v),
                 (wq_hbm, wq_v), (wo_hbm, wo_v), (w1_hbm, w1_v), (w2_hbm, w2_v)])]

        def start_head(h, slot):
            for isv, (src, buf) in enumerate([(k_hbm, kbuf), (v_hbm, vbuf)]):
                for j, (d0, s0) in enumerate(chunks):
                    pltpu.make_async_copy(
                        src.at[h, pl.ds(d0, CD), pl.ds(SK - W + s0, CS)],
                        buf.at[slot, pl.ds(d0, CD), pl.ds(s0, CS)],
                        sem_kv.at[isv, slot]).start(priority=j % 2)

        def wait_k(slot):
            pltpu.make_async_copy(kbuf.at[slot], kbuf.at[slot], sem_kv.at[0, slot]).wait()

        def wait_v(slot):
            pltpu.make_async_copy(vbuf.at[slot], vbuf.at[slot], sem_kv.at[1, slot]).wait()

        c_x.start()
        c_wq.start()
        start_head(0, 0)
        c_wo.start()
        c_gw.start()
        c_b1.start()
        c_b2.start()
        for i in range(1, NBUF):
            start_head(i, i)
        c_w1.start()
        c_w2.start()

        c_x.wait()
        c_wq.wait()
        x = x_v[...]
        xb = jnp.broadcast_to(x, (8, D))
        q = jnp.dot(xb, wq_v[...], preferred_element_type=_F32).astype(_BF16)
        for h in range(H):
            q_scr[h] = q[:, h * DH:(h + 1) * DH]
        c_wo.wait()

        def head(h, out_acc):
            slot = h % NBUF
            wait_k(slot)
            s = jnp.dot(q_scr[h], kbuf[slot], preferred_element_type=_F32)[0:1] * scale
            m = jnp.max(s, axis=1, keepdims=True)
            e = jnp.exp(s - m)
            l = jnp.sum(e, axis=1, keepdims=True)
            wait_v(slot)
            acc = jnp.zeros((DH, 128), _F32)
            for j in range(W // 128):
                acc = acc + vbuf[slot, :, j * 128:(j + 1) * 128].astype(_F32) * e[:, j * 128:(j + 1) * 128]
            o = jnp.sum(acc, axis=1, keepdims=True) * (1.0 / l)
            woh = wo_v[pl.ds(pl.multiple_of(h * DH, DH), DH), :].astype(_F32)
            out_acc = out_acc + (o * woh).reshape(DH // 8, 8, D).sum(axis=0)

            @pl.when(h + NBUF < H)
            def _():
                start_head(h + NBUF, slot)
            return out_acc

        out_acc = jax.lax.fori_loop(0, H, head, jnp.zeros((8, D), _F32))
        a = jnp.sum(out_acc, axis=0, keepdims=True)

        c_gw.wait()
        c_b1.wait()
        c_b2.wait()
        c_w1.wait()
        c_w2.wait()
        g = jax.nn.sigmoid(jnp.sum(x.astype(_F32) * gw_v[...].reshape(1, D).astype(_F32), axis=1, keepdims=True))
        hh = jnp.dot(xb, w1_v[...], preferred_element_type=_F32) + b1_v[...].reshape(1, F).astype(_F32)
        hh = _gelu(hh).astype(_BF16)
        b = (jnp.dot(hh, w2_v[...], preferred_element_type=_F32) + b2_v[...].reshape(1, D).astype(_F32))[0:1]
        o_ref[...] = (g * a + (1.0 - g) * b).astype(o_ref.dtype)

    kt = jnp.swapaxes(A_k_cache, 2, 3).reshape(H, DH, SK)
    vt = jnp.swapaxes(A_v_cache, 2, 3).reshape(H, DH, SK)
    out = pl.pallas_call(
        kernel,
        out_shape=jax.ShapeDtypeStruct((1, D), A_x.dtype),
        in_specs=[pl.BlockSpec(memory_space=pl.ANY)] * 10,
        out_specs=pl.BlockSpec(memory_space=pltpu.VMEM),
        scratch_shapes=[
            pltpu.VMEM((1, D), _BF16), pltpu.VMEM((D,), _BF16), pltpu.VMEM((F,), _BF16), pltpu.VMEM((D,), _BF16),
            pltpu.VMEM((D, H * DH), _BF16), pltpu.VMEM((H * DH, D), _BF16),
            pltpu.VMEM((D, F), _BF16), pltpu.VMEM((F, D), _BF16),
            pltpu.VMEM((NBUF, DH, W), _BF16), pltpu.VMEM((NBUF, DH, W), _BF16),
            pltpu.VMEM((H, 8, DH), _BF16),
            pltpu.SemaphoreType.DMA((8,)), pltpu.SemaphoreType.DMA((2, NBUF)),
        ],
        compiler_params=pltpu.CompilerParams(vmem_limit_bytes=100 * 1024 * 1024),
    )(A_x.reshape(1, D), gate_w, B_b1, B_b2, kt, vt, A_wq, A_wo, B_w1, B_w2)
    return out.reshape(1, 1, D)
```

```python
import functools
import jax
import jax.numpy as jnp
from jax.experimental import pallas as pl
from jax.experimental.pallas import tpu as pltpu

D, H, DH, SK, F = 640, 32, 192, 32768, 1536
W = min(4096, max(256, SK // 4))
bf16, f32 = jnp.bfloat16, jnp.float32
CS = 2048
CD = 8
NC = 48


def _gelu(x):
    c = 0.7978845608028654
    return 0.5 * x * (1.0 + jnp.tanh(c * (x + 0.044715 * (x * x * x))))


def kv_chunks(order):
    if order == 'ds':
        return [(d0, s0) for d0 in range(0, DH, CD) for s0 in range(0, W, CS)]
    return [(d0, s0) for s0 in range(0, W, CS) for d0 in range(0, DH, CD)]


def stride_order(n, S, d=1):
    out = []; used = set()
    for c in range(S):
        if c in used: continue
        if c + d < S and (c + d) not in used:
            pair = (c, c + d)
        else:
            pair = (c,)
        used.update(pair)
        for i in range((n + S - 1) // S):
            for cc in pair:
                a = i * S + cc
                if a < n: out.append(a)
    assert sorted(out) == list(range(n))
    return out


def make_kernel(nb=2, kvorder='sd', wqS=16, w1S=16, w2S=16, worows=24, compute=True):
    kvc = kv_chunks(kvorder)
    NWO = DH // worows
    stream = []
    w1o = stride_order(80, w1S) if w1S else list(range(80))
    stream += [('w1', rt * 8, 8, 0, F) for rt in w1o]
    w2o = stride_order(64, w2S) if w2S else list(range(64))
    stream += [('w2', i * 24, 24, 0, D) for i in w2o]
    for u in range(5):
        o = stride_order(48, wqS) if wqS else list(range(48))
        stream += [('wq', u * 128 + (a // 3) * 8, 8, (a % 3) * CS, CS) for a in o]
    NPRO = len(stream) // NC
    assert NPRO * NC == len(stream)

    def kernel(x_hbm, gw_hbm, b1_hbm, b2_hbm, k_hbm, v_hbm, wq_hbm, wo_hbm, w1_hbm, w2_hbm,
               o_ref,
               x_v, gw_v, b1_v, b2_v, wq_v, wo_v, w1_v, w2_v, kbuf, vbuf, q_scr,
               sem_s, sem_u, sem_wo):
        small = [pltpu.make_async_copy(s, d, sem_s.at[i]) for i, (s, d) in enumerate(
            [(x_hbm, x_v), (gw_hbm, gw_v), (b1_hbm, b1_v), (b2_hbm, b2_v)])]
        refs = dict(w1=(w1_hbm, w1_v), w2=(w2_hbm, w2_v), wq=(wq_hbm, wq_v))

        def d_pro(u, j):
            name, r0, nr, c0, nc = stream[u * NC + j]
            src, dst = refs[name]
            sl = (pl.ds(r0, nr), pl.ds(c0, nc))
            return pltpu.make_async_copy(src.at[sl], dst.at[sl], sem_u.at[u % nb, j])

        def d_kv(isv, h, j):
            src, buf = ((k_hbm, kbuf), (v_hbm, vbuf))[isv]
            slot = h % 2
            d0, s0 = kvc[j]
            return pltpu.make_async_copy(src.at[h, pl.ds(d0, 8), pl.ds(SK - W + s0, CS)],
                                         buf.at[slot, pl.ds(d0, 8), pl.ds(s0, CS)], sem_u.at[(NPRO + 2 * h + isv) % nb, j])

        def d_wo(h, j):
            slot = h % 2
            return pltpu.make_async_copy(wo_hbm.at[pl.ds(pl.multiple_of(h * DH + j * worows, 8), worows)],
                                         wo_v.at[slot, pl.ds(j * worows, worows)], sem_wo.at[slot, j])

        for c in small:
            c.start()
        for i in range(nb):
            for j in range(NC):
                d_pro(i, j).start(priority=j % 2)
        for c in small:
            c.wait()
        x = x_v[...]
        xb = jnp.broadcast_to(x, (8, D))
        q = jnp.zeros((8, H * DH), f32)
        for i in range(NPRO):
            nxt = i + nb
            if nxt - NPRO == 0:
                for j in range(NWO):
                    d_wo(0, j).start(priority=j % 2)
            for j in range(NC):
                d_pro(i, j).wait()
                if nxt < NPRO:
                    d_pro(nxt, j).start(priority=j % 2)
                else:
                    u = nxt - NPRO
                    d_kv(u % 2, u // 2, j).start(priority=j % 2)
            if i == 2:
                g = jax.nn.sigmoid(jnp.sum(x.astype(f32) * gw_v[...].reshape(1, D).astype(f32), axis=1, keepdims=True))
                hh = jnp.dot(xb, w1_v[...], preferred_element_type=f32) + b1_v[...].reshape(1, F).astype(f32)
                hh = _gelu(hh).astype(bf16)
                b = (jnp.dot(hh, w2_v[...], preferred_element_type=f32) + b2_v[...].reshape(1, D).astype(f32))[0:1]
                mixb = (1.0 - g) * b
            if i >= 3 and compute:
                ii = i - 3
                q = q + jnp.dot(xb[:, ii * 128:(ii + 1) * 128], wq_v[ii * 128:(ii + 1) * 128, :], preferred_element_type=f32)
        qb = q.astype(bf16)
        for h in range(H):
            q_scr[h] = qb[:, h * DH:(h + 1) * DH]

        scale = DH ** -0.5
        NU = 2 * H

        def head(h, out_acc):
            slot = h % 2
            for j in range(NC):
                d_kv(0, h, j).wait()
                @pl.when(2 * h + nb < NU)
                def _():
                    d_kv(nb % 2, (2 * h + nb) // 2, j).start(priority=j % 2)
            @pl.when(h + 1 < H)
            def _():
                for j in range(NWO):
                    d_wo(h + 1, j).start(priority=j % 2)
            if compute:
                qh = q_scr[h]
                s = jnp.dot(qh, kbuf[slot], preferred_element_type=f32)[0:1] * scale
                m = jnp.max(s, axis=1, keepdims=True)
                e = jnp.exp(s - m)
                l = jnp.sum(e, axis=1, keepdims=True)
            for j in range(NC):
                d_kv(1, h, j).wait()
                @pl.when(2 * h + 1 + nb < NU)
                def _():
                    d_kv((1 + nb) % 2, (2 * h + 1 + nb) // 2, j).start(priority=j % 2)
            for j in range(NWO):
                d_wo(h, j).wait()
            if compute:
                acc = jnp.zeros((DH, 128), f32)
                for j in range(W // 128):
                    acc = acc + vbuf[slot, :, j * 128:(j + 1) * 128].astype(f32) * e[:, j * 128:(j + 1) * 128]
                o = jnp.sum(acc, axis=1, keepdims=True) * (1.0 / l)
                woh = wo_v[slot].astype(f32)
                out_acc = out_acc + (o * woh).reshape(DH // 8, 8, D).sum(axis=0)
            return out_acc

        out_acc = jax.lax.fori_loop(0, H, head, jnp.zeros((8, D), f32))
        a = jnp.sum(out_acc, axis=0, keepdims=True)
        o_ref[...] = (g * a + mixb).astype(o_ref.dtype)

    def fn(A_x, A_k_cache, A_v_cache, A_wq, A_wo, B_x, B_w1, B_b1, B_w2, B_b2, gate_w):
        kt = jnp.swapaxes(A_k_cache, 2, 3).reshape(H, DH, SK)
        vt = jnp.swapaxes(A_v_cache, 2, 3).reshape(H, DH, SK)
        x2 = A_x.reshape(1, D)
        out = pl.pallas_call(
            kernel,
            out_shape=jax.ShapeDtypeStruct((1, D), bf16),
            in_specs=[pl.BlockSpec(memory_space=pl.ANY)] * 10,
            out_specs=pl.BlockSpec(memory_space=pltpu.VMEM),
            scratch_shapes=[
                pltpu.VMEM((1, D), bf16), pltpu.VMEM((D,), bf16), pltpu.VMEM((F,), bf16), pltpu.VMEM((D,), bf16),
                pltpu.VMEM((D, H * DH), bf16), pltpu.VMEM((2, DH, D), bf16),
                pltpu.VMEM((D, F), bf16), pltpu.VMEM((F, D), bf16),
                pltpu.VMEM((2, DH, W), bf16), pltpu.VMEM((2, DH, W), bf16),
                pltpu.VMEM((H, 8, DH), bf16),
                pltpu.SemaphoreType.DMA((4,)), pltpu.SemaphoreType.DMA((nb, NC)),
                pltpu.SemaphoreType.DMA((2, NWO)),
            ],
            compiler_params=pltpu.CompilerParams(vmem_limit_bytes=100 * 1024 * 1024, disable_bounds_checks=True),
        )(x2, gate_w, B_b1, B_b2, kt, vt, A_wq, A_wo, B_w1, B_w2)
        return out.reshape(1, 1, D)
    return fn


_FN = make_kernel(**dict(worows=192))


@jax.jit
def pallas_gated_mix__sliding_block_cached__dense_activation_gelu__decode_kernel(
    A_x, A_k_cache, A_v_cache, A_wq, A_wo, B_x, B_w1, B_b1, B_w2, B_b2, gate_w,
):
    return _FN(A_x, A_k_cache, A_v_cache, A_wq, A_wo, B_x, B_w1, B_b1, B_w2, B_b2, gate_w)
```

```python
import functools
import jax
import jax.numpy as jnp
from jax.experimental import pallas as pl
from jax.experimental.pallas import tpu as pltpu

D, H, DH, SK, F = 640, 32, 192, 32768, 1536
W = min(4096, max(256, SK // 4))
bf16, f32 = jnp.bfloat16, jnp.float32
CS = 2048


def _gelu(x):
    c = 0.7978845608028654
    return 0.5 * x * (1.0 + jnp.tanh(c * (x + 0.044715 * (x * x * x))))


def stride_order(n, S, d=1):
    if not S:
        return list(range(n))
    out = []; used = set()
    for c in range(S):
        if c in used: continue
        pair = (c, c + d) if (c + d < S and (c + d) not in used) else (c,)
        used.update(pair)
        for i in range((n + S - 1) // S):
            for cc in pair:
                a = i * S + cc
                if a < n: out.append(a)
    assert sorted(out) == list(range(n))
    return out


def make_kernel(win=96, korder='sd', vorder='sd', wqS=16, w1S=16, w2S=16, worows=192, wopos='mid', split=False, compute=True):
    def kvch(order):
        if order == 'ds':
            return [(d0, s0) for d0 in range(0, DH, 8) for s0 in range(0, W, CS)]
        return [(d0, s0) for s0 in range(0, W, CS) for d0 in range(0, DH, 8)]
    NWO = DH // worows
    pro = [('w1', rt * 8, 8, 0, F) for rt in stride_order(80, w1S)]
    pro += [('w2', i * 24, 24, 0, D) for i in stride_order(64, w2S)]
    for u in range(5):
        pro += [('wq', u * 128 + (a // 3) * 8, 8, (a % 3) * CS, CS) for a in stride_order(48, wqS)]
    NP = len(pro)
    ks = [('k',) + c for c in kvch(korder)]
    vs = [('v',) + c for c in kvch(vorder)]
    ws = [('wo', i * worows) for i in range(NWO)]
    if wopos == 'mid': hs = ks + ws + vs
    elif wopos == 'first': hs = ws + ks + vs
    elif wopos == 'last': hs = ks + vs + ws
    NH = len(hs)
    assert win <= NH
    k_end = max(j for j, c in enumerate(hs) if c[0] == 'k')
    k_mid = [j for j, c in enumerate(hs) if c[0] == 'k'][23]
    v_end = max(j for j, c in enumerate(hs) if c[0] == 'v')
    v_mid = [j for j, c in enumerate(hs) if c[0] == 'v'][23]
    w_end = max(j for j, c in enumerate(hs) if c[0] == 'wo')
    if split: assert korder == 'sd' and vorder == 'sd'

    def kernel(x_hbm, gw_hbm, b1_hbm, b2_hbm, k_hbm, v_hbm, wq_hbm, wo_hbm, w1_hbm, w2_hbm,
               o_ref,
               x_v, gw_v, b1_v, b2_v, wq_v, wo_v, w1_v, w2_v, kbuf, vbuf, q_scr,
               sem_s, sem_h):
        small = [pltpu.make_async_copy(s, d, sem_s.at[i]) for i, (s, d) in enumerate(
            [(x_hbm, x_v), (gw_hbm, gw_v), (b1_hbm, b1_v), (b2_hbm, b2_v)])]
        refs = dict(w1=(w1_hbm, w1_v), w2=(w2_hbm, w2_v), wq=(wq_hbm, wq_v))

        def d_pro(i):
            name, r0, nr, c0, nc = pro[i]
            src, dst = refs[name]
            sl = (pl.ds(r0, nr), pl.ds(c0, nc))
            return pltpu.make_async_copy(src.at[sl], dst.at[sl], sem_h.at[(i - NP) % NH])

        def d_head(h, j):
            c = hs[j]
            slot = h % 2
            if c[0] == 'wo':
                r0 = c[1]
                return pltpu.make_async_copy(wo_hbm.at[pl.ds(pl.multiple_of(h * DH + r0, 8), worows)],
                                             wo_v.at[slot, pl.ds(r0, worows)], sem_h.at[j])
            src, buf = (k_hbm, kbuf) if c[0] == 'k' else (v_hbm, vbuf)
            _, d0, s0 = c
            return pltpu.make_async_copy(src.at[h, pl.ds(d0, 8), pl.ds(SK - W + s0, CS)],
                                         buf.at[slot, pl.ds(d0, 8), pl.ds(s0, CS)], sem_h.at[j])

        def start_global(i):
            if i < NP:
                d_pro(i).start(priority=i % 2)
            else:
                d_head(0, i - NP).start(priority=(i - NP) % 2)

        for c in small:
            c.start()
        for i in range(win):
            start_global(i)
        for c in small:
            c.wait()
        x = x_v[...]
        xb = jnp.broadcast_to(x, (8, D))
        q = jnp.zeros((8, H * DH), f32)
        for i in range(NP):
            d_pro(i).wait()
            start_global(i + win)
            if i == 143:
                g = jax.nn.sigmoid(jnp.sum(x.astype(f32) * gw_v[...].reshape(1, D).astype(f32), axis=1, keepdims=True))
                hh = jnp.dot(xb, w1_v[...], preferred_element_type=f32) + b1_v[...].reshape(1, F).astype(f32)
                hh = _gelu(hh).astype(bf16)
                b = (jnp.dot(hh, w2_v[...], preferred_element_type=f32) + b2_v[...].reshape(1, D).astype(f32))[0:1]
                mixb = (1.0 - g) * b
            if i > 143 and (i - 143) % 48 == 0 and compute:
                ii = (i - 144) // 48
                q = q + jnp.dot(xb[:, ii * 128:(ii + 1) * 128], wq_v[ii * 128:(ii + 1) * 128, :], preferred_element_type=f32)
        qb = q.astype(bf16)
        for h in range(H):
            q_scr[h] = qb[:, h * DH:(h + 1) * DH]

        scale = DH ** -0.5

        def head(h, out_acc):
            slot = h % 2
            st = {}
            for j in range(NH):
                d_head(h, j).wait()
                jn = j + win
                if jn < NH:
                    d_head(h, jn).start(priority=jn % 2)
                else:
                    @pl.when(h + 1 < H)
                    def _():
                        d_head(h + 1, jn - NH).start(priority=jn % 2)
                if not compute:
                    continue
                if split:
                    if j == k_mid:
                        st['s0'] = jnp.dot(q_scr[h], kbuf[slot, :, 0:CS], preferred_element_type=f32)[0:1] * scale
                    if j == k_end:
                        s1 = jnp.dot(q_scr[h], kbuf[slot, :, CS:W], preferred_element_type=f32)[0:1] * scale
                        s0 = st['s0']
                        m = jnp.maximum(jnp.max(s0, axis=1, keepdims=True), jnp.max(s1, axis=1, keepdims=True))
                        st['e0'] = jnp.exp(s0 - m); st['e1'] = jnp.exp(s1 - m)
                        st['l'] = jnp.sum(st['e0'], axis=1, keepdims=True) + jnp.sum(st['e1'], axis=1, keepdims=True)
                    if j == v_mid:
                        acc = jnp.zeros((DH, 128), f32)
                        for t in range(CS // 128):
                            acc = acc + vbuf[slot, :, t * 128:(t + 1) * 128].astype(f32) * st['e0'][:, t * 128:(t + 1) * 128]
                        st['acc'] = acc
                    if j == v_end:
                        acc = st['acc']
                        for t in range(CS // 128):
                            acc = acc + vbuf[slot, :, CS + t * 128:CS + (t + 1) * 128].astype(f32) * st['e1'][:, t * 128:(t + 1) * 128]
                        st['o'] = jnp.sum(acc, axis=1, keepdims=True) * (1.0 / st['l'])
                else:
                    if j == k_end:
                        s = jnp.dot(q_scr[h], kbuf[slot], preferred_element_type=f32)[0:1] * scale
                        m = jnp.max(s, axis=1, keepdims=True)
                        st['e'] = jnp.exp(s - m)
                        st['l'] = jnp.sum(st['e'], axis=1, keepdims=True)
                    if j == v_end:
                        acc = jnp.zeros((DH, 128), f32)
                        for t in range(W // 128):
                            acc = acc + vbuf[slot, :, t * 128:(t + 1) * 128].astype(f32) * st['e'][:, t * 128:(t + 1) * 128]
                        st['o'] = jnp.sum(acc, axis=1, keepdims=True) * (1.0 / st['l'])
                if j == max(v_end, w_end):
                    woh = wo_v[slot].astype(f32)
                    out_acc = out_acc + (st['o'] * woh).reshape(DH // 8, 8, D).sum(axis=0)
            return out_acc

        out_acc = jax.lax.fori_loop(0, H, head, jnp.zeros((8, D), f32))
        a = jnp.sum(out_acc, axis=0, keepdims=True)
        o_ref[...] = (g * a + mixb).astype(o_ref.dtype)

    def fn(A_x, A_k_cache, A_v_cache, A_wq, A_wo, B_x, B_w1, B_b1, B_w2, B_b2, gate_w):
        kt = jnp.swapaxes(A_k_cache, 2, 3).reshape(H, DH, SK)
        vt = jnp.swapaxes(A_v_cache, 2, 3).reshape(H, DH, SK)
        x2 = A_x.reshape(1, D)
        out = pl.pallas_call(
            kernel,
            out_shape=jax.ShapeDtypeStruct((1, D), bf16),
            in_specs=[pl.BlockSpec(memory_space=pl.ANY)] * 10,
            out_specs=pl.BlockSpec(memory_space=pltpu.VMEM),
            scratch_shapes=[
                pltpu.VMEM((1, D), bf16), pltpu.VMEM((D,), bf16), pltpu.VMEM((F,), bf16), pltpu.VMEM((D,), bf16),
                pltpu.VMEM((D, H * DH), bf16), pltpu.VMEM((2, DH, D), bf16),
                pltpu.VMEM((D, F), bf16), pltpu.VMEM((F, D), bf16),
                pltpu.VMEM((2, DH, W), bf16), pltpu.VMEM((2, DH, W), bf16),
                pltpu.VMEM((H, 8, DH), bf16),
                pltpu.SemaphoreType.DMA((4,)),
                pltpu.SemaphoreType.DMA((NH,)),
            ],
            compiler_params=pltpu.CompilerParams(vmem_limit_bytes=100 * 1024 * 1024, disable_bounds_checks=True, disable_semaphore_checks=True),
        )(x2, gate_w, B_b1, B_b2, kt, vt, A_wq, A_wo, B_w1, B_w2)
        return out.reshape(1, 1, D)
    return fn


_FN = make_kernel(**dict(worows=48,split=True,wopos='last'))


@jax.jit
def pallas_gated_mix__sliding_block_cached__dense_activation_gelu__decode_kernel(
    A_x, A_k_cache, A_v_cache, A_wq, A_wo, B_x, B_w1, B_b1, B_w2, B_b2, gate_w,
):
    return _FN(A_x, A_k_cache, A_v_cache, A_wq, A_wo, B_x, B_w1, B_b1, B_w2, B_b2, gate_w)
```

```python
import jax
import jax.numpy as jnp
from jax.experimental import pallas as pl
from jax.experimental.pallas import tpu as pltpu

D, H, DH, SK, F = 640, 32, 192, 32768, 1536
W = min(4096, max(256, SK // 4))
bf16, f32 = jnp.bfloat16, jnp.float32
CS = 2048


def _gelu(x):
    c = 0.7978845608028654
    return 0.5 * x * (1.0 + jnp.tanh(c * (x + 0.044715 * (x * x * x))))


def stride_order(n, S, d=1):
    if not S:
        return list(range(n))
    out = []; used = set()
    for c in range(S):
        if c in used: continue
        pair = (c, c + d) if (c + d < S and (c + d) not in used) else (c,)
        used.update(pair)
        for i in range((n + S - 1) // S):
            for cc in pair:
                a = i * S + cc
                if a < n: out.append(a)
    assert sorted(out) == list(range(n))
    return out


def make_kernel(win=96, wqS=16, w1S=16, w2S=16, worows=48, worows_last=48, vsplit=(2048, 2048), vsplit_last=(2048, 2048),
                peel=True, compute=True, wo_hooks=True):
    R = range(0, DH, 8)
    ks = [('k', d0, s0, CS) for s0 in range(0, W, CS) for d0 in R]
    def vstream(sp):
        out = []; s = 0
        for w in sp:
            out += [('v', d0, s, w) for d0 in R]; s += w
        assert s == W
        return out
    def ws(rows): return [('wo', r0, rows) for r0 in range(0, DH, rows)]
    def spread(kv, w):
        out = []; step = len(kv) // len(w); k = 0
        for i, c in enumerate(kv):
            out.append(c)
            if (i + 1) % step == 0 and k < len(w):
                out.append(w[k]); k += 1
        return out
    hs_main = spread(ks + vstream(vsplit), ws(worows))
    hs_last = ks + vstream(vsplit_last) + ws(worows_last) if peel else hs_main
    NSEM = max(len(hs_main), len(hs_last))
    assert win <= min(len(hs_main), len(hs_last))

    pro = [('w1', rt * 8, 8, 0, F) for rt in stride_order(80, w1S)]
    pro += [('w2', i * 24, 24, 0, D) for i in stride_order(64, w2S)]
    for u in range(5):
        pro += [('wq', u * 128 + (a // 3) * 8, 8, (a % 3) * CS, CS) for a in stride_order(48, wqS)]
    NP = len(pro)

    def kernel(x_hbm, gw_hbm, b1_hbm, b2_hbm, k_hbm, v_hbm, wq_hbm, wo_hbm, w1_hbm, w2_hbm,
               o_ref,
               x_v, gw_v, b1_v, b2_v, wq_v, wo_v, w1_v, w2_v, kbuf, vbuf, q_scr,
               sem_s, sem_h):
        small = [pltpu.make_async_copy(s, d, sem_s.at[i]) for i, (s, d) in enumerate(
            [(x_hbm, x_v), (gw_hbm, gw_v), (b1_hbm, b1_v), (b2_hbm, b2_v)])]
        refs = dict(w1=(w1_hbm, w1_v), w2=(w2_hbm, w2_v), wq=(wq_hbm, wq_v))

        def d_pro(i):
            name, r0, nr, c0, nc = pro[i]
            src, dst = refs[name]
            sl = (pl.ds(r0, nr), pl.ds(c0, nc))
            return pltpu.make_async_copy(src.at[sl], dst.at[sl], sem_h.at[(i - NP) % len(hs_main)])

        def d_head(h, hs, j):
            c = hs[j]
            slot = h % 2
            if c[0] == 'wo':
                _, r0, rows = c
                row = h * DH + r0
                if not isinstance(row, int):
                    row = pl.multiple_of(row, 8)
                return pltpu.make_async_copy(wo_hbm.at[pl.ds(row, rows)], wo_v.at[slot, pl.ds(r0, rows)], sem_h.at[j])
            src, buf = (k_hbm, kbuf) if c[0] == 'k' else (v_hbm, vbuf)
            _, d0, s0, w = c
            return pltpu.make_async_copy(src.at[h, pl.ds(d0, 8), pl.ds(SK - W + s0, w)],
                                         buf.at[slot, pl.ds(d0, 8), pl.ds(s0, w)], sem_h.at[j])

        def start_global(i):
            if i < NP:
                d_pro(i).start(priority=i % 2)
            else:
                d_head(0, hs_main, i - NP).start(priority=(i - NP) % 2)

        for i in range(4):
            start_global(i)
        for c in small:
            c.start()
        for i in range(4, win):
            start_global(i)
        for c in small:
            c.wait()
        x = x_v[...]
        xb = jnp.broadcast_to(x, (8, D))
        q = jnp.zeros((8, H * DH), f32)
        for i in range(NP):
            d_pro(i).wait()
            start_global(i + win)
            if i == 143:
                g = jax.nn.sigmoid(jnp.sum(x.astype(f32) * gw_v[...].reshape(1, D).astype(f32), axis=1, keepdims=True))
                hh = jnp.dot(xb, w1_v[...], preferred_element_type=f32) + b1_v[...].reshape(1, F).astype(f32)
                hh = _gelu(hh).astype(bf16)
                b = (jnp.dot(hh, w2_v[...], preferred_element_type=f32) + b2_v[...].reshape(1, D).astype(f32))[0:1]
                mixb = (1.0 - g) * b
            if i > 143 and (i - 143) % 48 == 0 and compute:
                ii = (i - 144) // 48
                q = q + jnp.dot(xb[:, ii * 128:(ii + 1) * 128], wq_v[ii * 128:(ii + 1) * 128, :], preferred_element_type=f32)
        qb = q.astype(bf16)
        for h in range(H):
            q_scr[h] = qb[:, h * DH:(h + 1) * DH]

        scale = DH ** -0.5

        def head(h, out_acc, hs, hs_next, dyn_guard):
            slot = h % 2
            NH = len(hs)
            kpos = [j for j, c in enumerate(hs) if c[0] == 'k']
            k_mid, k_end = kpos[len(kpos) // 2 - 1], kpos[-1]
            vseg = {}
            for j, c in enumerate(hs):
                if c[0] == 'v':
                    vseg[(c[2], c[3])] = j
            vhook = {j: seg for seg, j in vseg.items()}
            v_end = max(vhook)
            wpos = [j for j, c in enumerate(hs) if c[0] == 'wo']
            st = {}
            for j in range(NH):
                d_head(h, hs, j).wait()
                jn = j + win
                if jn < NH:
                    d_head(h, hs, jn).start(priority=jn % 2)
                elif hs_next is not None:
                    if dyn_guard:
                        @pl.when(h + 1 < H)
                        def _():
                            d_head(h + 1, hs_next, jn - NH).start(priority=(jn - NH) % 2)
                    else:
                        d_head(h + 1, hs_next, jn - NH).start(priority=(jn - NH) % 2)
                if not compute:
                    continue
                if j == k_mid:
                    st['s0'] = jnp.dot(q_scr[h], kbuf[slot, :, 0:CS], preferred_element_type=f32)[0:1] * scale
                if j == k_end:
                    s1 = jnp.dot(q_scr[h], kbuf[slot, :, CS:W], preferred_element_type=f32)[0:1] * scale
                    s0 = st['s0']
                    m = jnp.maximum(jnp.max(s0, axis=1, keepdims=True), jnp.max(s1, axis=1, keepdims=True))
                    st['e'] = jnp.concatenate([jnp.exp(s0 - m), jnp.exp(s1 - m)], axis=1)
                    st['il'] = 1.0 / jnp.sum(st['e'], axis=1, keepdims=True)
                if j in vhook:
                    s0_, w_ = vhook[j]
                    acc = st.get('acc')
                    if acc is None:
                        acc = jnp.zeros((DH, 128), f32)
                    for t in range(s0_ // 128, (s0_ + w_) // 128):
                        acc = acc + vbuf[slot, :, t * 128:(t + 1) * 128].astype(f32) * st['e'][:, t * 128:(t + 1) * 128]
                    st['acc'] = acc
                    if j == v_end:
                        st['o'] = jnp.sum(acc, axis=1, keepdims=True) * st['il']
                if wpos[0] > v_end and wo_hooks:
                    if j in wpos:
                        _, r0, rows = hs[j]
                        woh = wo_v[slot, r0:r0 + rows, :].astype(f32)
                        out_acc = out_acc + (st['o'][r0:r0 + rows] * woh).reshape(rows // 8, 8, D).sum(axis=0)
                elif j == max(v_end, wpos[-1]):
                    woh = wo_v[slot].astype(f32)
                    out_acc = out_acc + (st['o'] * woh).reshape(DH // 8, 8, D).sum(axis=0)
            return out_acc

        out_acc = jnp.zeros((8, D), f32)
        if peel:
            out_acc = jax.lax.fori_loop(0, H - 2, lambda h, a: head(h, a, hs_main, hs_main, False), out_acc)
            out_acc = head(H - 2, out_acc, hs_main, hs_last, False)
            out_acc = head(H - 1, out_acc, hs_last, None, False)
        else:
            out_acc = jax.lax.fori_loop(0, H, lambda h, a: head(h, a, hs_main, hs_main, True), out_acc)
        a = jnp.sum(out_acc, axis=0, keepdims=True)
        o_ref[...] = (g * a + mixb).astype(o_ref.dtype)

    def fn(A_x, A_k_cache, A_v_cache, A_wq, A_wo, B_x, B_w1, B_b1, B_w2, B_b2, gate_w):
        kt = jnp.swapaxes(A_k_cache, 2, 3).reshape(H, DH, SK)
        vt = jnp.swapaxes(A_v_cache, 2, 3).reshape(H, DH, SK)
        x2 = A_x.reshape(1, D)
        out = pl.pallas_call(
            kernel,
            out_shape=jax.ShapeDtypeStruct((1, D), bf16),
            in_specs=[pl.BlockSpec(memory_space=pl.ANY)] * 10,
            out_specs=pl.BlockSpec(memory_space=pltpu.VMEM),
            scratch_shapes=[
                pltpu.VMEM((1, D), bf16), pltpu.VMEM((D,), bf16), pltpu.VMEM((F,), bf16), pltpu.VMEM((D,), bf16),
                pltpu.VMEM((D, H * DH), bf16), pltpu.VMEM((2, DH, D), bf16),
                pltpu.VMEM((D, F), bf16), pltpu.VMEM((F, D), bf16),
                pltpu.VMEM((2, DH, W), bf16), pltpu.VMEM((2, DH, W), bf16),
                pltpu.VMEM((H, 8, DH), bf16),
                pltpu.SemaphoreType.DMA((4,)),
                pltpu.SemaphoreType.DMA((NSEM,)),
            ],
            compiler_params=pltpu.CompilerParams(vmem_limit_bytes=100 * 1024 * 1024, disable_bounds_checks=True, disable_semaphore_checks=True),
        )(x2, gate_w, B_b1, B_b2, kt, vt, A_wq, A_wo, B_w1, B_w2)
        return out.reshape(1, 1, D)
    return fn


_FN = make_kernel(**dict(vsplit_last=(2048,1024,512,512)))


@jax.jit
def pallas_gated_mix__sliding_block_cached__dense_activation_gelu__decode_kernel(
    A_x, A_k_cache, A_v_cache, A_wq, A_wo, B_x, B_w1, B_b1, B_w2, B_b2, gate_w,
):
    return _FN(A_x, A_k_cache, A_v_cache, A_wq, A_wo, B_x, B_w1, B_b1, B_w2, B_b2, gate_w)
```

```python
import jax
import jax.numpy as jnp
import jax.experimental.pallas as pl
import jax.experimental.pallas.tpu as pltpu

_BF16 = jnp.bfloat16
_F32 = jnp.float32

_WIN = 96
_CS = 2048
_WO_ROWS = 48
_W2_ROWS = 24
_V_SPLIT = (2048, 2048)
_V_SPLIT_LAST = (2048, 1024, 512, 512)
_STRIDE = 16


def _gelu(x):
    c = 0.7978845608028654
    return 0.5 * x * (1.0 + jnp.tanh(c * (x + 0.044715 * (x * x * x))))


def _stride_order(n, stride):
    out = []
    for c in range(0, stride, 2):
        for i in range(-(-n // stride)):
            out += [a for a in (i * stride + c, i * stride + c + 1) if a < n]
    return out


def _spread(base, extra):
    step = len(base) // len(extra)
    out = []
    for i, c in enumerate(base):
        out.append(c)
        if (i + 1) % step == 0 and (i + 1) // step <= len(extra):
            out.append(extra[(i + 1) // step - 1])
    return out


@jax.jit
def pallas_gated_mix__sliding_block_cached__dense_activation_gelu__decode_kernel(
    A_x: jax.Array,
    A_k_cache: jax.Array,
    A_v_cache: jax.Array,
    A_wq: jax.Array,
    A_wo: jax.Array,
    B_x: jax.Array,
    B_w1: jax.Array,
    B_b1: jax.Array,
    B_w2: jax.Array,
    B_b2: jax.Array,
    gate_w: jax.Array,
):
    del B_x
    D = A_x.shape[-1]
    _, H, SK, DH = A_k_cache.shape
    F = B_w1.shape[1]
    W = min(4096, max(256, SK // 4))
    assert W == sum(_V_SPLIT) == sum(_V_SPLIT_LAST) == 2 * _CS
    assert A_wq.shape == (D, H * DH) and H * DH == 3 * _CS and D % 128 == 0
    scale = DH ** -0.5

    rows = range(0, DH, 8)
    k_chunks = [("k", d0, s0, _CS) for s0 in range(0, W, _CS) for d0 in rows]

    def v_chunks(split):
        out, s0 = [], 0
        for w in split:
            out += [("v", d0, s0, w) for d0 in rows]
            s0 += w
        return out

    wo_chunks = [("wo", r0, _WO_ROWS) for r0 in range(0, DH, _WO_ROWS)]
    hs_main = _spread(k_chunks + v_chunks(_V_SPLIT), wo_chunks)
    hs_last = k_chunks + v_chunks(_V_SPLIT_LAST) + wo_chunks
    n_sem = max(len(hs_main), len(hs_last))
    assert _WIN <= min(len(hs_main), len(hs_last))

    pro = [("w1", t * 8, 8, 0, F) for t in _stride_order(D // 8, _STRIDE)]
    pro += [("w2", t * _W2_ROWS, _W2_ROWS, 0, D) for t in _stride_order(F // _W2_ROWS, _STRIDE)]
    ffn_pos = len(pro) - 1
    q_pos = {}
    per_row = H * DH // _CS
    for u in range(D // 128):
        pro += [("wq", u * 128 + (a // per_row) * 8, 8, (a % per_row) * _CS, _CS)
                for a in _stride_order(16 * per_row, _STRIDE)]
        q_pos[len(pro) - 1] = u
    n_pro = len(pro)

    def kernel(x_hbm, gw_hbm, b1_hbm, b2_hbm, k_hbm, v_hbm, wq_hbm, wo_hbm, w1_hbm, w2_hbm,
               o_ref,
               x_v, gw_v, b1_v, b2_v, wq_v, wo_v, w1_v, w2_v, kbuf, vbuf, q_scr, sem_s, sem):
        small = [pltpu.make_async_copy(s, d, sem_s.at[i]) for i, (s, d) in enumerate(
            [(x_hbm, x_v), (gw_hbm, gw_v), (b1_hbm, b1_v), (b2_hbm, b2_v)])]
        weights = dict(w1=(w1_hbm, w1_v), w2=(w2_hbm, w2_v), wq=(wq_hbm, wq_v))

        def pro_copy(i):
            name, r0, nr, c0, nc = pro[i]
            src, dst = weights[name]
            idx = (pl.ds(r0, nr), pl.ds(c0, nc))
            return pltpu.make_async_copy(src.at[idx], dst.at[idx], sem.at[(i - n_pro) % len(hs_main)])

        def head_copy(h, hs, j):
            c = hs[j]
            slot = h % 2
            if c[0] == "wo":
                _, r0, nr = c
                row = h * DH + r0
                if not isinstance(row, int):
                    row = pl.multiple_of(row, 8)
                return pltpu.make_async_copy(
                    wo_hbm.at[pl.ds(row, nr)], wo_v.at[slot, pl.ds(r0, nr)], sem.at[j])
            src, buf = (k_hbm, kbuf) if c[0] == "k" else (v_hbm, vbuf)
            _, d0, s0, w = c
            return pltpu.make_async_copy(
                src.at[h, pl.ds(d0, 8), pl.ds(SK - W + s0, w)],
                buf.at[slot, pl.ds(d0, 8), pl.ds(s0, w)], sem.at[j])

        def start_pro(i):
            if i < n_pro:
                pro_copy(i).start(priority=i % 2)
            else:
                head_copy(0, hs_main, i - n_pro).start(priority=(i - n_pro) % 2)

        for i in range(4):
            start_pro(i)
        for c in small:
            c.start()
        for i in range(4, _WIN):
            start_pro(i)
        for c in small:
            c.wait()
        x = x_v[...]
        xb = jnp.broadcast_to(x, (8, D))
        q = jnp.zeros((8, H * DH), _F32)
        for i in range(n_pro):
            pro_copy(i).wait()
            start_pro(i + _WIN)
            if i == ffn_pos:
                g = jax.nn.sigmoid(jnp.sum(
                    x.astype(_F32) * gw_v[...].reshape(1, D).astype(_F32), axis=1, keepdims=True))
                hid = jnp.dot(xb, w1_v[...], preferred_element_type=_F32)
                hid = _gelu(hid + b1_v[...].reshape(1, F).astype(_F32)).astype(_BF16)
                b = jnp.dot(hid, w2_v[...], preferred_element_type=_F32)
                b = (b + b2_v[...].reshape(1, D).astype(_F32))[0:1]
                mix_b = (1.0 - g) * b
            if i in q_pos:
                u = q_pos[i]
                q = q + jnp.dot(xb[:, u * 128:(u + 1) * 128], wq_v[u * 128:(u + 1) * 128, :],
                                preferred_element_type=_F32)
        qb = q.astype(_BF16)
        for h in range(H):
            q_scr[h] = qb[:, h * DH:(h + 1) * DH]

        def head(h, out_acc, hs, hs_next):
            slot = h % 2
            n = len(hs)
            k_pos = [j for j, c in enumerate(hs) if c[0] == "k"]
            k_mid, k_end = k_pos[len(k_pos) // 2 - 1], k_pos[-1]
            v_seg = {(c[2], c[3]): j for j, c in enumerate(hs) if c[0] == "v"}
            v_hook = {j: seg for seg, j in v_seg.items()}
            v_end = max(v_hook)
            wo_pos = [j for j, c in enumerate(hs) if c[0] == "wo"]
            st = {}
            for j in range(n):
                head_copy(h, hs, j).wait()
                jn = j + _WIN
                if jn < n:
                    head_copy(h, hs, jn).start(priority=jn % 2)
                elif hs_next is not None:
                    head_copy(h + 1, hs_next, jn - n).start(priority=(jn - n) % 2)

                if j == k_mid:
                    st["s0"] = jnp.dot(q_scr[h], kbuf[slot, :, 0:_CS],
                                       preferred_element_type=_F32)[0:1] * scale
                if j == k_end:
                    s0 = st["s0"]
                    s1 = jnp.dot(q_scr[h], kbuf[slot, :, _CS:W],
                                 preferred_element_type=_F32)[0:1] * scale
                    m = jnp.maximum(jnp.max(s0, axis=1, keepdims=True),
                                    jnp.max(s1, axis=1, keepdims=True))
                    st["e"] = jnp.concatenate([jnp.exp(s0 - m), jnp.exp(s1 - m)], axis=1)
                    st["inv_l"] = 1.0 / jnp.sum(st["e"], axis=1, keepdims=True)
                if j in v_hook:
                    c0, w = v_hook[j]
                    acc = st.get("acc")
                    if acc is None:
                        acc = jnp.zeros((DH, 128), _F32)
                    for t in range(c0 // 128, (c0 + w) // 128):
                        cols = slice(t * 128, (t + 1) * 128)
                        acc = acc + vbuf[slot, :, cols].astype(_F32) * st["e"][:, cols]
                    st["acc"] = acc
                    if j == v_end:
                        st["o"] = jnp.sum(acc, axis=1, keepdims=True) * st["inv_l"]
                if wo_pos[0] > v_end:
                    if j in wo_pos:
                        _, r0, nr = hs[j]
                        woh = wo_v[slot, r0:r0 + nr, :].astype(_F32)
                        out_acc = out_acc + (st["o"][r0:r0 + nr] * woh).reshape(nr // 8, 8, D).sum(axis=0)
                elif j == max(v_end, wo_pos[-1]):
                    woh = wo_v[slot].astype(_F32)
                    out_acc = out_acc + (st["o"] * woh).reshape(DH // 8, 8, D).sum(axis=0)
            return out_acc

        out_acc = jnp.zeros((8, D), _F32)
        out_acc = jax.lax.fori_loop(
            0, H - 2, lambda h, a: head(h, a, hs_main, hs_main), out_acc)
        out_acc = head(H - 2, out_acc, hs_main, hs_last)
        out_acc = head(H - 1, out_acc, hs_last, None)
        a = jnp.sum(out_acc, axis=0, keepdims=True)
        o_ref[...] = (g * a + mix_b).astype(o_ref.dtype)

    kt = jnp.swapaxes(A_k_cache, 2, 3).reshape(H, DH, SK)
    vt = jnp.swapaxes(A_v_cache, 2, 3).reshape(H, DH, SK)
    out = pl.pallas_call(
        kernel,
        out_shape=jax.ShapeDtypeStruct((1, D), A_x.dtype),
        in_specs=[pl.BlockSpec(memory_space=pl.ANY)] * 10,
        out_specs=pl.BlockSpec(memory_space=pltpu.VMEM),
        scratch_shapes=[
            pltpu.VMEM((1, D), _BF16), pltpu.VMEM((D,), _BF16),
            pltpu.VMEM((F,), _BF16), pltpu.VMEM((D,), _BF16),
            pltpu.VMEM((D, H * DH), _BF16), pltpu.VMEM((2, DH, D), _BF16),
            pltpu.VMEM((D, F), _BF16), pltpu.VMEM((F, D), _BF16),
            pltpu.VMEM((2, DH, W), _BF16), pltpu.VMEM((2, DH, W), _BF16),
            pltpu.VMEM((H, 8, DH), _BF16),
            pltpu.SemaphoreType.DMA((4,)),
            pltpu.SemaphoreType.DMA((n_sem,)),
        ],
        compiler_params=pltpu.CompilerParams(
            vmem_limit_bytes=100 * 1024 * 1024,
            disable_bounds_checks=True,
            disable_semaphore_checks=True,
        ),
    )(A_x.reshape(1, D), gate_w, B_b1, B_b2, kt, vt, A_wq, A_wo, B_w1, B_w2)
    return out.reshape(1, 1, D)
```
